```python
import os as _os
_os.environ.setdefault('JAX_PLATFORMS', 'cpu')
import jax
import jax.numpy as jnp

def _softmax(x, axis=-1):
    return jax.nn.softmax(x, axis=axis)

def _gelu(x):
    return jax.nn.gelu(x, approximate=True)

def _silu(x):
    return jax.nn.silu(x)

def _sigmoid(x):
    return jax.nn.sigmoid(x)

def _layernorm(x, axis=-1, eps=1e-05):
    m = jnp.mean(x, axis=axis, keepdims=True)
    v = jnp.var(x, axis=axis, keepdims=True)
    return (x - m) / jnp.sqrt(v + eps)

def _scatter_add(tgt, idx, src, axis=0):
    return tgt.at[idx].add(src)

def _segment_sum(src, seg, n):
    return jax.ops.segment_sum(src, seg, n)

class _Rng:

    def __init__(self, key):
        self._k = key

    def _next(self):
        self._k, sub = jax.random.split(self._k)
        return sub

    def normal(self, shape):
        return jax.random.normal(self._next(), shape, dtype=jnp.bfloat16)

    def randint(self, lo, hi, shape):
        return jax.random.randint(self._next(), shape, lo, hi, dtype=jnp.int32)

    def uniform(self, shape, lo=0.0, hi=1.0):
        return jax.random.uniform(self._next(), shape, jnp.bfloat16, lo, hi)

    def permutation(self, n):
        return jax.random.permutation(self._next(), n)
kernel_name = 'adaLN_cond__mha_block__geglu_ffn__prompt'

def setup_inputs():
    _rng = _Rng(jax.random.key(int.from_bytes(__import__("os").urandom(4), "little")))
    _w = lambda a: (lambda t: t.astype(jnp.bfloat16) if jnp.issubdtype(t.dtype, jnp.floating) else t)(jnp.asarray(a))

    def _A_setup():
        B, S, D, H = (1, 2048, 640, 32)
        return {'x': _w((lambda *s: _rng.normal(s) * 0.05)(B, S, D)), 'wqkv': _w((lambda *s: _rng.normal(s) * 0.05)(D, 3 * D)), 'wo': _w((lambda *s: _rng.normal(s) * 0.05)(D, D))}
    _A_in = _A_setup()

    def _B_setup():
        B, S, D, F = (1, 2048, 640, 1728)
        return {'x': _w((lambda *s: _rng.normal(s) * 0.05)(B, S, D)), 'w_gate': _w((lambda *s: _rng.normal(s) * 0.05)(D, F)), 'w_up': _w((lambda *s: _rng.normal(s) * 0.05)(D, F)), 'w_down': _w((lambda *s: _rng.normal(s) * 0.05)(F, D))}
    _B_in = _B_setup()
    return {'A_x': _A_in['x'], 'A_wqkv': _A_in['wqkv'], 'A_wo': _A_in['wo'], 'B_x': _B_in['x'], 'B_w_gate': _B_in['w_gate'], 'B_w_up': _B_in['w_up'], 'B_w_down': _B_in['w_down'], 'c': _w((lambda *s: _rng.normal(s) * 0.05)(1, 640) * 8.0), 'w_mod': _w((lambda *s: _rng.normal(s) * 0.05)(640, 6 * 640) * 640 ** (-0.5) * 8.0)}

def reference(A_x, A_wqkv, A_wo, B_x, B_w_gate, B_w_up, B_w_down, c, w_mod):

    def _A_ref(x, wqkv, wo):
        B, S, D = x.shape
        H = 32
        Dh = D // H
        qkv = (lambda x, *d: x.transpose(*d))((x @ wqkv).reshape(B, S, 3, H, Dh), 2, 0, 3, 1, 4)
        q, k, v = (qkv[0], qkv[1], qkv[2])
        scores = jnp.einsum('bhqd,bhkd->bhqk', q, k) * Dh ** (-0.5)
        p = _softmax(scores, axis=-1)
        o = jnp.einsum('bhqk,bhkd->bhqd', p, v)
        return (lambda x, *d: x.transpose(*d))(o, 0, 2, 1, 3).reshape(B, S, D) @ wo

    def _B_ref(x, w_gate, w_up, w_down):
        return _gelu(x @ w_gate) * (x @ w_up) @ w_down
    x = A_x
    mod = (_silu(c) @ w_mod).reshape(c.shape[0], 6, 1, -1)
    sa, ca, ga, sb, cb, gb = (mod[:, 0].copy(), mod[:, 1].copy(), mod[:, 2].copy(), mod[:, 3].copy(), mod[:, 4].copy(), mod[:, 5].copy())
    h = _layernorm(x, axis=-1) * (1 + ca) + sa
    x = x + ga * _A_ref(h, A_wqkv, A_wo)
    h = _layernorm(x, axis=-1) * (1 + cb) + sb
    x = x + gb * _B_ref(h, B_w_gate, B_w_up, B_w_down)
    return x
```

```python
import functools
import math

import jax
import jax.numpy as jnp
import jax.experimental.pallas as pl
import jax.experimental.pallas.tpu as pltpu

H = 32
DH = 20
EPS = 1e-5
LANES = 128
HEADS_PER_WIN = 6
VROWS = 32
TQ = 512
CK = 128

_BF = jnp.bfloat16
_F32 = jnp.float32
_NT = (((1,), (1,)), ((), ()))


def _layernorm(x):
    m = jnp.mean(x, axis=-1, keepdims=True)
    xc = x - m
    v = jnp.mean(xc * xc, axis=-1, keepdims=True)
    return xc * jax.lax.rsqrt(v + EPS)


def _gelu_tanh(x):
    c = math.sqrt(2.0 / math.pi)
    return 0.5 * x * (1.0 + jnp.tanh(c * (x + 0.044715 * (x * x * x))))


def _win_start(g, d_model):
    return min(g * HEADS_PER_WIN * DH, d_model - LANES)


def _kernel(x_hbm, wqkv_hbm, wo_hbm, wg_hbm, wu_hbm, wd_hbm, c_ref, wmod_hbm,
            o_ref,
            x_v, wqkv_v, wo_v, wg_v, wu_v, wd_v, wmod_v,
            mod_v, wqt_v, wvt_v, wkw_v, k_v, vt_v, qt_v,
            sa_v, sb_v, ma_v, mb_v, ot_v, sems,
            *, S, D, F):
    step = pl.program_id(0)
    nblk = S // TQ
    nwin = -(-H // HEADS_PER_WIN)
    qscale = (DH ** -0.5) * math.log2(math.e)

    def copies():
        pairs = [(wmod_hbm, wmod_v), (x_hbm, x_v), (wqkv_hbm, wqkv_v), (wo_hbm, wo_v),
                 (wg_hbm, wg_v), (wu_hbm, wu_v), (wd_hbm, wd_v)]
        return [pltpu.make_async_copy(s, d, sems.at[i]) for i, (s, d) in enumerate(pairs)]

    def qmask(blk, head):
        g = head // HEADS_PER_WIN
        start = jnp.minimum(g * (HEADS_PER_WIN * DH), D - LANES)
        base = head * DH - start
        qt = qt_v[blk, pl.ds(pl.multiple_of(start, 8), LANES), :]
        row = jax.lax.broadcasted_iota(jnp.int32, (LANES, TQ), 0)
        qm = jnp.where((row >= base) & (row < base + DH), qt, 0.0).astype(_BF)
        return g, qm

    def qk_chunk(g, qm, c, s_ref, mpart):
        rows = slice(c * CK, (c + 1) * CK)
        s = jnp.dot(k_v[g, rows, :], qm, preferred_element_type=_F32)
        s_ref[rows, :] = s
        mp = jnp.max(s.reshape(CK // 8, 8, TQ), axis=0)
        return mp if mpart is None else jnp.maximum(mpart, mp)

    def phase(blk_n, head_n, sn_ref, mn_ref, head_c, sc_ref, mc_ref):
        g, qm = qmask(blk_n, head_n)
        mcur = mc_ref[...]
        mpart = None
        acc = None
        for c in range(S // CK):
            rows = slice(c * CK, (c + 1) * CK)
            mpart = qk_chunk(g, qm, c, sn_ref, mpart)
            p = jnp.exp2(sc_ref[rows, :] - mcur).astype(_BF)
            part = jnp.dot(vt_v[head_c, :, rows], p, preferred_element_type=_F32)
            acc = part if acc is None else acc + part
        mn_ref[...] = jnp.max(mpart, axis=0, keepdims=True)
        return acc[0:DH] / acc[DH:DH + 1]

    @pl.when(step == 0)
    def _prologue():
        cps = copies()
        for cp in cps:
            cp.start()
        c = c_ref[...].astype(_F32)
        sc = (c * jax.nn.sigmoid(c)).astype(_BF)
        sc8 = jnp.broadcast_to(sc, (8, D))
        cps[0].wait()
        mod_v[...] = jnp.dot(sc8, wmod_v[...], preferred_element_type=_F32)
        cps[2].wait()
        wqt_v[...] = wqkv_v[:, 0:D].T
        wvt_v[...] = wqkv_v[:, 2 * D:3 * D].T
        for g in range(nwin):
            st = D + _win_start(g, D)
            wkw_v[:, g * LANES:(g + 1) * LANES] = wqkv_v[:, st:st + LANES]
        cps[1].wait()
        shift = mod_v[0:1, 0:D]
        scale = 1.0 + mod_v[0:1, D:2 * D]

        def proj(b, carry):
            r0 = pl.multiple_of(b * TQ, TQ)
            x = x_v[pl.ds(r0, TQ), :].astype(_F32)
            h = (_layernorm(x) * scale + shift).astype(_BF)
            kk = jnp.dot(h, wkw_v[...], preferred_element_type=_F32)
            for g in range(nwin):
                k_v[g, pl.ds(r0, TQ), :] = kk[:, g * LANES:(g + 1) * LANES].astype(_BF)
            nt = (((1,), (1,)), ((), ()))
            qt = jax.lax.dot_general(wqt_v[...], h, nt, preferred_element_type=_F32)
            qt_v[b] = qt * qscale
            vt = jax.lax.dot_general(wvt_v[...], h, nt, preferred_element_type=_F32)
            rowi = jax.lax.broadcasted_iota(jnp.int32, (VROWS - DH, TQ), 0)
            tail = jnp.where(rowi == 0, 1.0, 0.0).astype(_F32)
            for hh in range(H):
                slab = jnp.concatenate([vt[hh * DH:(hh + 1) * DH], tail], axis=0)
                vt_v[hh, :, pl.ds(r0, TQ)] = slab.astype(_BF)
            return carry

        jax.lax.fori_loop(0, nblk, proj, 0)
        g, qm = qmask(0, 0)
        mpart = None
        for c in range(S // CK):
            mpart = qk_chunk(g, qm, c, sa_v, mpart)
        ma_v[...] = jnp.max(mpart, axis=0, keepdims=True)
        for cp in cps[3:]:
            cp.wait()

    def pair(j, carry):
        h0 = 2 * j
        oa = phase(step, h0 + 1, sb_v, mb_v, h0, sa_v, ma_v)
        nxt = h0 + 2
        wrap = nxt // H
        ob = phase(jnp.minimum(step + wrap, nblk - 1), nxt - wrap * H, sa_v, ma_v, h0 + 1, sb_v, mb_v)
        ot_v[pl.ds(pl.multiple_of(2 * DH * j, 8), 2 * DH), :] = jnp.concatenate([oa, ob], axis=0)
        return carry

    jax.lax.fori_loop(0, H // 2, pair, 0)

    r0 = pl.multiple_of(step * TQ, TQ)
    o = ot_v[...].T.astype(_BF)
    attn = jnp.dot(o, wo_v[...], preferred_element_type=_F32)
    x1 = x_v[pl.ds(r0, TQ), :].astype(_F32) + mod_v[0:1, 2 * D:3 * D] * attn
    h2 = (_layernorm(x1) * (1.0 + mod_v[0:1, 4 * D:5 * D]) + mod_v[0:1, 3 * D:4 * D]).astype(_BF)
    acc = None
    FC = 512
    for f0 in range(0, F, FC):
        f1 = min(f0 + FC, F)
        gate = jax.lax.dot_general(h2, wg_v[f0:f1, :], _NT, preferred_element_type=_F32)
        up = jax.lax.dot_general(h2, wu_v[f0:f1, :], _NT, preferred_element_type=_F32)
        act = (_gelu_tanh(gate) * up).astype(_BF)
        part = jnp.dot(act, wd_v[f0:f1, :], preferred_element_type=_F32)
        acc = part if acc is None else acc + part
    o_ref[...] = (x1 + mod_v[0:1, 5 * D:6 * D] * acc).astype(o_ref.dtype)


@jax.jit
def pallas_adaLN_cond__mha_block__geglu_ffn__prompt_kernel(
    A_x: jax.Array,
    A_wqkv: jax.Array,
    A_wo: jax.Array,
    B_x: jax.Array,
    B_w_gate: jax.Array,
    B_w_up: jax.Array,
    B_w_down: jax.Array,
    c: jax.Array,
    w_mod: jax.Array,
):
    B, S, D = A_x.shape
    F = B_w_gate.shape[1]
    assert B == 1 and D == H * DH and S % TQ == 0
    nblk = S // TQ
    nwin = -(-H // HEADS_PER_WIN)
    x2 = A_x.reshape(S, D)

    hbm = pl.BlockSpec(memory_space=pltpu.HBM)
    scratch = [
        pltpu.VMEM((S, D), _BF),
        pltpu.VMEM((D, 3 * D), _BF),
        pltpu.VMEM((D, D), _BF),
        pltpu.VMEM((F, D), _BF),
        pltpu.VMEM((F, D), _BF),
        pltpu.VMEM((F, D), _BF),
        pltpu.VMEM((D, 6 * D), _BF),
        pltpu.VMEM((8, 6 * D), _F32),
        pltpu.VMEM((D, D), _BF),
        pltpu.VMEM((D, D), _BF),
        pltpu.VMEM((D, nwin * LANES), _BF),
        pltpu.VMEM((nwin, S, LANES), _BF),
        pltpu.VMEM((H, VROWS, S), _BF),
        pltpu.VMEM((nblk, D, TQ), _F32),
        pltpu.VMEM((S, TQ), _F32),
        pltpu.VMEM((S, TQ), _F32),
        pltpu.VMEM((1, TQ), _F32),
        pltpu.VMEM((1, TQ), _F32),
        pltpu.VMEM((D, TQ), _F32),
        pltpu.SemaphoreType.DMA((7,)),
    ]
    out = pl.pallas_call(
        functools.partial(_kernel, S=S, D=D, F=F),
        grid=(nblk,),
        in_specs=[hbm, hbm, hbm, hbm, hbm, hbm,
                  pl.BlockSpec((1, D), lambda i: (0, 0)),
                  hbm],
        out_specs=pl.BlockSpec((TQ, D), lambda i: (i, 0)),
        out_shape=jax.ShapeDtypeStruct((S, D), A_x.dtype),
        scratch_shapes=scratch,
        compiler_params=pltpu.CompilerParams(
            dimension_semantics=("arbitrary",),
            vmem_limit_bytes=100 * 1024 * 1024,
        ),
    )(x2, A_wqkv, A_wo, B_w_gate.T, B_w_up.T, B_w_down, c, w_mod)
    return out.reshape(B, S, D)
```

```python
import functools
import math

import jax
import jax.numpy as jnp
import jax.experimental.pallas as pl
import jax.experimental.pallas.tpu as pltpu

H = 32
DH = 20
EPS = 1e-5
LANES = 128
HEADS_PER_WIN = 6
VROWS = 32
TQ = 512
CK = 128
LAG = 4
FC = 512
NH = 8
PIN = 4

_BF = jnp.bfloat16
_F32 = jnp.float32
_NT = (((1,), (1,)), ((), ()))


def _layernorm(x):
    m = jnp.mean(x, axis=-1, keepdims=True)
    xc = x - m
    v = jnp.mean(xc * xc, axis=-1, keepdims=True)
    return xc * jax.lax.rsqrt(v + EPS)


def _gelu_tanh(x):
    c = math.sqrt(2.0 / math.pi)
    return 0.5 * x * (1.0 + jnp.tanh(c * (x + 0.044715 * (x * x * x))))


def _win_start(g, d_model):
    return min(g * HEADS_PER_WIN * DH, d_model - LANES)


def _kernel(x_hbm, wqkv_hbm, wo_hbm, wg_hbm, wu_hbm, wd_hbm, c_hbm, wmod_hbm,
            o_ref,
            x_v, wqkv_v, wo_v, wg_v, wu_v, wd_v, c_v, wmod_v,
            mod_v, h_v, wqt_v, wvt_v, k_v, vt_v, qt_v,
            sa_v, sb_v, ma_v, ot_v, sems,
            *, S, D, F):
    step = pl.program_id(0)
    nblk = S // TQ
    nch = S // CK
    nwin = -(-H // HEADS_PER_WIN)
    qscale = (DH ** -0.5) * math.log2(math.e)

    def cp_c():
        return pltpu.make_async_copy(c_hbm, c_v, sems.at[0])

    def cp_wk():
        return pltpu.make_async_copy(wqkv_hbm.at[:, pl.ds(D, D)], wqkv_v.at[:, pl.ds(D, D)], sems.at[1])

    def cp_wq():
        return pltpu.make_async_copy(wqkv_hbm.at[:, pl.ds(0, D)], wqkv_v.at[:, pl.ds(0, D)], sems.at[8 + nblk])

    def cp_wv():
        return pltpu.make_async_copy(wqkv_hbm.at[:, pl.ds(2 * D, D)], wqkv_v.at[:, pl.ds(2 * D, D)],
                                     sems.at[9 + nblk])

    def cp_mod_a():
        return pltpu.make_async_copy(wmod_hbm.at[:, pl.ds(0, 2 * D)], wmod_v.at[:, pl.ds(0, 2 * D)], sems.at[2])

    def cp_mod_b():
        return pltpu.make_async_copy(wmod_hbm.at[:, pl.ds(2 * D, 4 * D)], wmod_v.at[:, pl.ds(2 * D, 4 * D)],
                                     sems.at[3])

    def cp_late():
        pairs = [(wo_hbm, wo_v), (wg_hbm, wg_v), (wu_hbm, wu_v), (wd_hbm, wd_v)]
        return [pltpu.make_async_copy(s, d, sems.at[4 + i]) for i, (s, d) in enumerate(pairs)]

    def cp_x(b):
        r0 = pl.multiple_of(b * TQ, TQ)
        return pltpu.make_async_copy(x_hbm.at[pl.ds(r0, TQ)], x_v.at[pl.ds(r0, TQ)], sems.at[8 + b])

    def qmask(blk, head):
        g = head // HEADS_PER_WIN
        start = jnp.minimum(g * (HEADS_PER_WIN * DH), D - LANES)
        base = head * DH - start
        qt = qt_v[blk, pl.ds(pl.multiple_of(start, 8), LANES), :]
        row = jax.lax.broadcasted_iota(jnp.int32, (LANES, TQ), 0)
        qm = jnp.where((row >= base) & (row < base + DH), qt, 0.0).astype(_BF)
        return g, qm

    def qk_chunk(g, qm, c, s_ref, mpart):
        rows = slice(c * CK, (c + 1) * CK)
        s = jnp.dot(k_v[g, rows, :], qm, preferred_element_type=_F32)
        s_ref[rows, :] = s
        mp = jnp.max(s.reshape(CK // 8, 8, TQ), axis=0)
        return mp if mpart is None else jnp.maximum(mpart, mp)

    @pl.when(step == 0)
    def _prologue():
        cp_c().start()
        cp_mod_a().start()
        cp_x(0).start()
        cp_wk().start()
        cp_c().wait()
        cp_mod_a().wait()
        c = c_v[...].astype(_F32)
        sc8 = jnp.broadcast_to((c * jax.nn.sigmoid(c)).astype(_BF), (8, D))
        mod_v[:, 0:2 * D] = jnp.dot(sc8, wmod_v[:, 0:2 * D], preferred_element_type=_F32)
        shift = mod_v[0:1, 0:D]
        scale = 1.0 + mod_v[0:1, D:2 * D]
        cp_wk().wait()
        for b in range(1, nblk):
            cp_x(b).start()
        cp_wq().start()
        cp_wv().start()
        cp_mod_b().start()
        for cp in cp_late():
            cp.start()

        def proj_k(b, carry):
            cp_x(b).wait()
            for hf in range(2):
                r0 = pl.multiple_of(b * TQ + hf * (TQ // 2), TQ // 2)
                rows = pl.ds(r0, TQ // 2)
                x = x_v[rows, :].astype(_F32)
                h = (_layernorm(x) * scale + shift).astype(_BF)
                h_v[rows, :] = h
                kk = jnp.dot(h, wqkv_v[:, D:2 * D], preferred_element_type=_F32)
                for g in range(nwin):
                    st = _win_start(g, D)
                    k_v[g, rows, :] = kk[:, st:st + LANES].astype(_BF)
            return carry

        jax.lax.fori_loop(0, nblk, proj_k, 0)

        cp_wq().wait()
        cp_wv().wait()
        cp_mod_b().wait()
        wqt_v[...] = wqkv_v[:, 0:D].T
        wvt_v[...] = wqkv_v[:, 2 * D:3 * D].T
        mod_v[:, 2 * D:6 * D] = jnp.dot(sc8, wmod_v[:, 2 * D:6 * D], preferred_element_type=_F32)

        def proj_qv(b, carry):
            r0 = pl.multiple_of(b * TQ, TQ)
            h = h_v[pl.ds(r0, TQ), :]
            qt = jax.lax.dot_general(wqt_v[...], h, _NT, preferred_element_type=_F32)
            qt_v[b] = qt * qscale
            vt = jax.lax.dot_general(wvt_v[...], h, _NT, preferred_element_type=_F32)
            rowi = jax.lax.broadcasted_iota(jnp.int32, (VROWS - DH, TQ), 0)
            tail = jnp.where(rowi == 0, 1.0, 0.0).astype(_F32)
            for hh in range(H):
                slab = jnp.concatenate([vt[hh * DH:(hh + 1) * DH], tail], axis=0)
                vt_v[hh, :, pl.ds(r0, TQ)] = slab.astype(_BF)
            return carry

        jax.lax.fori_loop(0, nblk, proj_qv, 0)
        g, qm = qmask(0, 0)
        mpart = None
        for c_ in range(nch):
            mpart = qk_chunk(g, qm, c_, sa_v, mpart)
        ma_v[...] = jnp.max(mpart, axis=0, keepdims=True)
        for cp in cp_late():
            cp.wait()

    def heads(j, carry):
        h0 = NH * j
        sw = [sb_v, sa_v] * (NH // 2)
        sr = [sa_v, sb_v] * (NH // 2)
        qk = [None] * NH
        m = [ma_v[...]] + [None] * (NH - 1)
        mpart = [None] * NH
        acc = [None] * NH
        pins = {}
        pv_at = {}
        for i in range(NH):
            for c_ in range(nch):
                t = i * nch + LAG + (c_ if i < NH - 1 else (c_ * (nch - LAG)) // nch)
                pv_at.setdefault(t, []).append((i, c_))
        for t in range(NH * nch):
            i, c_ = divmod(t, nch)
            if c_ == 0:
                nxt = h0 + 1 + i
                if i == NH - 1:
                    wrap = nxt // H
                    qk[i] = qmask(jnp.minimum(step + wrap, nblk - 1), nxt - wrap * H)
                else:
                    qk[i] = qmask(step, nxt)
            mpart[i] = qk_chunk(qk[i][0], qk[i][1], c_, sw[i], mpart[i])
            pins[t] = mpart[i]
            if c_ == nch - 1:
                mfin = jnp.max(mpart[i], axis=0, keepdims=True)
                if i < NH - 1:
                    m[i + 1] = mfin
                else:
                    ma_v[...] = mfin
            for i, c_ in pv_at.get(t, []):
                rows = slice(c_ * CK, (c_ + 1) * CK)
                mu = m[i]
                if (t - PIN) in pins:
                    mu = jnp.maximum(mu, jnp.minimum(pins[t - PIN][0:1, :], mu))
                p = jnp.exp2(sr[i][rows, :] - mu).astype(_BF)
                part = jnp.dot(vt_v[h0 + i, :, rows], p, preferred_element_type=_F32)
                acc[i] = part if acc[i] is None else acc[i] + part
                if c_ == nch - 1 and i % 2 == 1:
                    oa = acc[i - 1][0:DH] / acc[i - 1][DH:DH + 1]
                    ob = acc[i][0:DH] / acc[i][DH:DH + 1]
                    ot_v[pl.ds(pl.multiple_of(DH * (h0 + i - 1), 8), 2 * DH), :] = jnp.concatenate([oa, ob], axis=0)
        return carry

    jax.lax.fori_loop(0, H // NH, heads, 0)

    HT = TQ // 2
    ga = mod_v[0:1, 2 * D:3 * D]
    shift2 = mod_v[0:1, 3 * D:4 * D]
    scale2 = 1.0 + mod_v[0:1, 4 * D:5 * D]
    gb = mod_v[0:1, 5 * D:6 * D]
    x1 = []
    h2 = []
    for hf in range(2):
        r0 = pl.multiple_of(step * TQ + hf * HT, HT)
        o = ot_v[:, hf * HT:(hf + 1) * HT].T.astype(_BF)
        attn = jnp.dot(o, wo_v[...], preferred_element_type=_F32)
        xh = x_v[pl.ds(r0, HT), :].astype(_F32) + ga * attn
        x1.append(xh)
        h2.append((_layernorm(xh) * scale2 + shift2).astype(_BF))

    def gate_up(hh, f0, f1):
        gate = jax.lax.dot_general(hh, wg_v[f0:f1, :], _NT, preferred_element_type=_F32)
        up = jax.lax.dot_general(hh, wu_v[f0:f1, :], _NT, preferred_element_type=_F32)
        return (_gelu_tanh(gate) * up).astype(_BF)

    bounds = list(range(0, F, FC)) + [F]
    h2f = jnp.concatenate(h2, axis=0)
    acts = []
    for ci in range(len(bounds) - 1):
        f0, f1 = bounds[ci], bounds[ci + 1]
        if ci == 0:
            act = jnp.concatenate([gate_up(h2[0], f0, f1), gate_up(h2[1], f0, f1)], axis=0)
        elif (f1 - f0) % LANES == LANES // 2:
            fm = f1 - LANES // 2
            wt = jnp.concatenate([wg_v[fm:f1, :], wu_v[fm:f1, :]], axis=0)
            gu = jax.lax.dot_general(h2f, wt, _NT, preferred_element_type=_F32)
            tail = (_gelu_tanh(gu[:, 0:LANES // 2]) * gu[:, LANES // 2:LANES]).astype(_BF)
            act = jnp.concatenate([gate_up(h2f, f0, fm), tail], axis=1)
        else:
            act = gate_up(h2f, f0, f1)
        acts.append(act)
    acc = None
    for ci in range(len(bounds) - 2):
        part = jnp.dot(acts[ci], wd_v[bounds[ci]:bounds[ci + 1], :], preferred_element_type=_F32)
        acc = part if acc is None else acc + part
    for hf in range(2):
        rs = slice(hf * HT, (hf + 1) * HT)
        part = jnp.dot(acts[-1][rs], wd_v[bounds[-2]:bounds[-1], :], preferred_element_type=_F32)
        o_ref[rs, :] = (x1[hf] + gb * (acc[rs] + part)).astype(o_ref.dtype)


@jax.jit
def pallas_adaLN_cond__mha_block__geglu_ffn__prompt_kernel(
    A_x: jax.Array,
    A_wqkv: jax.Array,
    A_wo: jax.Array,
    B_x: jax.Array,
    B_w_gate: jax.Array,
    B_w_up: jax.Array,
    B_w_down: jax.Array,
    c: jax.Array,
    w_mod: jax.Array,
):
    B, S, D = A_x.shape
    F = B_w_gate.shape[1]
    assert B == 1 and D == H * DH and S % TQ == 0
    nblk = S // TQ
    nwin = -(-H // HEADS_PER_WIN)
    x2 = A_x.reshape(S, D)

    hbm = pl.BlockSpec(memory_space=pltpu.HBM)
    scratch = [
        pltpu.VMEM((S, D), _BF),
        pltpu.VMEM((D, 3 * D), _BF),
        pltpu.VMEM((D, D), _BF),
        pltpu.VMEM((F, D), _BF),
        pltpu.VMEM((F, D), _BF),
        pltpu.VMEM((F, D), _BF),
        pltpu.VMEM((1, D), _BF),
        pltpu.VMEM((D, 6 * D), _BF),
        pltpu.VMEM((8, 6 * D), _F32),
        pltpu.VMEM((S, D), _BF),
        pltpu.VMEM((D, D), _BF),
        pltpu.VMEM((D, D), _BF),
        pltpu.VMEM((nwin, S, LANES), _BF),
        pltpu.VMEM((H, VROWS, S), _BF),
        pltpu.VMEM((nblk, D, TQ), _F32),
        pltpu.VMEM((S, TQ), _F32),
        pltpu.VMEM((S, TQ), _F32),
        pltpu.VMEM((1, TQ), _F32),
        pltpu.VMEM((D, TQ), _F32),
        pltpu.SemaphoreType.DMA((10 + nblk,)),
    ]
    out = pl.pallas_call(
        functools.partial(_kernel, S=S, D=D, F=F),
        grid=(nblk,),
        in_specs=[hbm] * 8,
        out_specs=pl.BlockSpec((TQ, D), lambda i: (i, 0)),
        out_shape=jax.ShapeDtypeStruct((S, D), A_x.dtype),
        scratch_shapes=scratch,
        compiler_params=pltpu.CompilerParams(
            dimension_semantics=("arbitrary",),
            vmem_limit_bytes=100 * 1024 * 1024,
        ),
    )(x2, A_wqkv, A_wo, B_w_gate.T, B_w_up.T, B_w_down, c, w_mod)
    return out.reshape(B, S, D)
```

```python
import functools
import math

import jax
import jax.numpy as jnp
import jax.experimental.pallas as pl
import jax.experimental.pallas.tpu as pltpu

H = 32
DH = 20
EPS = 1e-5
LANES = 128
HEADS_PER_WIN = 6
VROWS = 32
TQ = 512
CK = 128
LAG = 4
FC = 512
NH = 8
PIN = 4

_BF = jnp.bfloat16
_F32 = jnp.float32
_NT = (((1,), (1,)), ((), ()))


def _layernorm(x):
    m = jnp.mean(x, axis=-1, keepdims=True)
    xc = x - m
    v = jnp.mean(xc * xc, axis=-1, keepdims=True)
    return xc * jax.lax.rsqrt(v + EPS)


def _gelu_tanh(x):
    c = math.sqrt(2.0 / math.pi)
    return 0.5 * x * (1.0 + jnp.tanh(c * (x + 0.044715 * (x * x * x))))


def _win_start(g, d_model):
    return min(g * HEADS_PER_WIN * DH, d_model - LANES)


def _kernel(x_hbm, wqkv_hbm, wo_hbm, wg_hbm, wu_hbm, wd_hbm, c_hbm, wmod_hbm,
            o_ref,
            x_v, wq_v, wk_v, wv_v, wo_v, wg_v, wu_v, wd_v, c_v, wma_v, wmb_v,
            mod_v, h_v, wqt_v, wvt_v, k_v, vt_v, qt_v,
            sa_v, sb_v, ma_v, ot_v, sems,
            *, S, D, F):
    step = pl.program_id(0)
    nblk = S // TQ
    nch = S // CK
    nwin = -(-H // HEADS_PER_WIN)
    qscale = (DH ** -0.5) * math.log2(math.e)

    def cp_c():
        return pltpu.make_async_copy(c_hbm, c_v, sems.at[0])

    def cp_wk():
        return pltpu.make_async_copy(wqkv_hbm.at[:, pl.ds(D, D)], wk_v, sems.at[1])

    def cp_wq():
        return pltpu.make_async_copy(wqkv_hbm.at[:, pl.ds(0, D)], wq_v, sems.at[8 + nblk])

    def cp_wv():
        return pltpu.make_async_copy(wqkv_hbm.at[:, pl.ds(2 * D, D)], wv_v, sems.at[9 + nblk])

    def cp_mod_a():
        return pltpu.make_async_copy(wmod_hbm.at[:, pl.ds(0, 2 * D)], wma_v, sems.at[2])

    def cp_mod_b():
        return pltpu.make_async_copy(wmod_hbm.at[:, pl.ds(2 * D, 4 * D)], wmb_v, sems.at[3])

    def cp_late():
        pairs = [(wo_hbm, wo_v), (wg_hbm, wg_v), (wu_hbm, wu_v), (wd_hbm, wd_v)]
        return [pltpu.make_async_copy(s, d, sems.at[4 + i]) for i, (s, d) in enumerate(pairs)]

    def cp_x(b):
        r0 = pl.multiple_of(b * TQ, TQ)
        return pltpu.make_async_copy(x_hbm.at[pl.ds(r0, TQ)], x_v.at[pl.ds(r0, TQ)], sems.at[8 + b])

    def qmask(blk, head):
        g = head // HEADS_PER_WIN
        start = jnp.minimum(g * (HEADS_PER_WIN * DH), D - LANES)
        base = head * DH - start
        qt = qt_v[blk, pl.ds(pl.multiple_of(start, 8), LANES), :]
        row = jax.lax.broadcasted_iota(jnp.int32, (LANES, TQ), 0)
        qm = jnp.where((row >= base) & (row < base + DH), qt, 0.0).astype(_BF)
        return g, qm

    def qk_chunk(g, qm, c, s_ref, mpart):
        rows = slice(c * CK, (c + 1) * CK)
        s = jnp.dot(k_v[g, rows, :], qm, preferred_element_type=_F32)
        s_ref[rows, :] = s
        mp = jnp.max(s.reshape(CK // 8, 8, TQ), axis=0)
        return mp if mpart is None else jnp.maximum(mpart, mp)

    @pl.when(step == 0)
    def _prologue():
        cp_c().start()
        cp_mod_a().start()
        cp_x(0).start()
        cp_wk().start()
        cp_c().wait()
        cp_mod_a().wait()
        c = c_v[...].astype(_F32)
        sc8 = jnp.broadcast_to((c * jax.nn.sigmoid(c)).astype(_BF), (8, D))
        mod_v[:, 0:2 * D] = jnp.dot(sc8, wma_v[...], preferred_element_type=_F32)
        shift = mod_v[0:1, 0:D]
        scale = 1.0 + mod_v[0:1, D:2 * D]
        cp_wk().wait()
        for b in range(1, nblk):
            cp_x(b).start()
        cp_wq().start()
        cp_wv().start()
        cp_mod_b().start()
        for cp in cp_late():
            cp.start()

        def proj_k(b, carry):
            cp_x(b).wait()
            for hf in range(2):
                r0 = pl.multiple_of(b * TQ + hf * (TQ // 2), TQ // 2)
                rows = pl.ds(r0, TQ // 2)
                x = x_v[rows, :].astype(_F32)
                h = (_layernorm(x) * scale + shift).astype(_BF)
                h_v[rows, :] = h
                kk = jnp.dot(h, wk_v[...], preferred_element_type=_F32)
                for g in range(nwin):
                    st = _win_start(g, D)
                    k_v[g, rows, :] = kk[:, st:st + LANES].astype(_BF)
            return carry

        jax.lax.fori_loop(0, nblk, proj_k, 0)

        cp_wq().wait()
        cp_wv().wait()
        cp_mod_b().wait()
        wqt_v[...] = wq_v[...].T
        wvt_v[...] = wv_v[...].T
        mod_v[:, 2 * D:6 * D] = jnp.dot(sc8, wmb_v[...], preferred_element_type=_F32)

        def proj_qv(b, carry):
            r0 = pl.multiple_of(b * TQ, TQ)
            h = h_v[pl.ds(r0, TQ), :]
            qt = jax.lax.dot_general(wqt_v[...], h, _NT, preferred_element_type=_F32)
            qt_v[b] = qt * qscale
            vt = jax.lax.dot_general(wvt_v[...], h, _NT, preferred_element_type=_F32)
            rowi = jax.lax.broadcasted_iota(jnp.int32, (VROWS - DH, TQ), 0)
            tail = jnp.where(rowi == 0, 1.0, 0.0).astype(_F32)
            for hh in range(H):
                slab = jnp.concatenate([vt[hh * DH:(hh + 1) * DH], tail], axis=0)
                vt_v[hh, :, pl.ds(r0, TQ)] = slab.astype(_BF)
            return carry

        jax.lax.fori_loop(0, nblk, proj_qv, 0)
        g, qm = qmask(0, 0)
        mpart = None
        for c_ in range(nch):
            mpart = qk_chunk(g, qm, c_, sa_v, mpart)
        ma_v[...] = jnp.max(mpart, axis=0, keepdims=True)
        for cp in cp_late():
            cp.wait()

    def heads(j, carry):
        h0 = NH * j
        sw = [sb_v, sa_v] * (NH // 2)
        sr = [sa_v, sb_v] * (NH // 2)
        qk = [None] * NH
        m = [ma_v[...]] + [None] * (NH - 1)
        mpart = [None] * NH
        acc = [None] * NH
        pins = {}
        pv_at = {}
        for i in range(NH):
            for c_ in range(nch):
                t = i * nch + LAG + (c_ if i < NH - 1 else (c_ * (nch - LAG)) // nch)
                pv_at.setdefault(t, []).append((i, c_))
        for t in range(NH * nch):
            i, c_ = divmod(t, nch)
            if c_ == 0:
                nxt = h0 + 1 + i
                if i == NH - 1:
                    wrap = nxt // H
                    qk[i] = qmask(jnp.minimum(step + wrap, nblk - 1), nxt - wrap * H)
                else:
                    qk[i] = qmask(step, nxt)
            mpart[i] = qk_chunk(qk[i][0], qk[i][1], c_, sw[i], mpart[i])
            if i < NH - 1:
                pins[t] = mpart[i]
            if c_ == nch - 1:
                mfin = jnp.max(mpart[i], axis=0, keepdims=True)
                if i < NH - 1:
                    m[i + 1] = mfin
                else:
                    ma_v[...] = mfin
            for i, c_ in pv_at.get(t, []):
                rows = slice(c_ * CK, (c_ + 1) * CK)
                mu = m[i]
                if (t - PIN) in pins:
                    mu = jnp.maximum(mu, jnp.minimum(pins[t - PIN][0:1, :], mu))
                p = jnp.exp2(sr[i][rows, :] - mu).astype(_BF)
                part = jnp.dot(vt_v[h0 + i, :, rows], p, preferred_element_type=_F32)
                acc[i] = part if acc[i] is None else acc[i] + part
                if c_ == nch - 1 and i % 2 == 1:
                    oa = acc[i - 1][0:DH] / acc[i - 1][DH:DH + 1]
                    ob = acc[i][0:DH] / acc[i][DH:DH + 1]
                    ot_v[pl.ds(pl.multiple_of(DH * (h0 + i - 1), 8), 2 * DH), :] = jnp.concatenate([oa, ob], axis=0)
        return carry

    jax.lax.fori_loop(0, H // NH, heads, 0)

    HT = TQ // 2
    ga = mod_v[0:1, 2 * D:3 * D]
    shift2 = mod_v[0:1, 3 * D:4 * D]
    scale2 = 1.0 + mod_v[0:1, 4 * D:5 * D]
    gb = mod_v[0:1, 5 * D:6 * D]
    x1 = []
    h2 = []
    for hf in range(2):
        r0 = pl.multiple_of(step * TQ + hf * HT, HT)
        o = ot_v[:, hf * HT:(hf + 1) * HT].T.astype(_BF)
        attn = jnp.dot(o, wo_v[...], preferred_element_type=_F32)
        xh = x_v[pl.ds(r0, HT), :].astype(_F32) + ga * attn
        x1.append(xh)
        h2.append((_layernorm(xh) * scale2 + shift2).astype(_BF))

    def gate_up(hh, f0, f1):
        gate = jax.lax.dot_general(hh, wg_v[f0:f1, :], _NT, preferred_element_type=_F32)
        up = jax.lax.dot_general(hh, wu_v[f0:f1, :], _NT, preferred_element_type=_F32)
        return (_gelu_tanh(gate) * up).astype(_BF)

    bounds = list(range(0, F, FC)) + [F]
    h2f = jnp.concatenate(h2, axis=0)
    acts = []
    for ci in range(len(bounds) - 1):
        f0, f1 = bounds[ci], bounds[ci + 1]
        if ci == 0:
            act = jnp.concatenate([gate_up(h2[0], f0, f1), gate_up(h2[1], f0, f1)], axis=0)
        elif (f1 - f0) % LANES == LANES // 2:
            fm = f1 - LANES // 2
            wt = jnp.concatenate([wg_v[fm:f1, :], wu_v[fm:f1, :]], axis=0)
            gu = jax.lax.dot_general(h2f, wt, _NT, preferred_element_type=_F32)
            tail = (_gelu_tanh(gu[:, 0:LANES // 2]) * gu[:, LANES // 2:LANES]).astype(_BF)
            act = jnp.concatenate([gate_up(h2f, f0, fm), tail], axis=1)
        else:
            act = gate_up(h2f, f0, f1)
        acts.append(act)
    acc = None
    for ci in range(len(bounds) - 2):
        part = jnp.dot(acts[ci], wd_v[bounds[ci]:bounds[ci + 1], :], preferred_element_type=_F32)
        acc = part if acc is None else acc + part
    for hf in range(2):
        rs = slice(hf * HT, (hf + 1) * HT)
        part = jnp.dot(acts[-1][rs], wd_v[bounds[-2]:bounds[-1], :], preferred_element_type=_F32)
        o_ref[rs, :] = (x1[hf] + gb * (acc[rs] + part)).astype(o_ref.dtype)


@jax.jit
def pallas_adaLN_cond__mha_block__geglu_ffn__prompt_kernel(
    A_x: jax.Array,
    A_wqkv: jax.Array,
    A_wo: jax.Array,
    B_x: jax.Array,
    B_w_gate: jax.Array,
    B_w_up: jax.Array,
    B_w_down: jax.Array,
    c: jax.Array,
    w_mod: jax.Array,
):
    B, S, D = A_x.shape
    F = B_w_gate.shape[1]
    assert B == 1 and D == H * DH and S % TQ == 0
    nblk = S // TQ
    nwin = -(-H // HEADS_PER_WIN)
    x2 = A_x.reshape(S, D)

    hbm = pl.BlockSpec(memory_space=pltpu.HBM)
    scratch = [
        pltpu.VMEM((S, D), _BF),
        pltpu.VMEM((D, D), _BF),
        pltpu.VMEM((D, D), _BF),
        pltpu.VMEM((D, D), _BF),
        pltpu.VMEM((D, D), _BF),
        pltpu.VMEM((F, D), _BF),
        pltpu.VMEM((F, D), _BF),
        pltpu.VMEM((F, D), _BF),
        pltpu.VMEM((1, D), _BF),
        pltpu.VMEM((D, 2 * D), _BF),
        pltpu.VMEM((D, 4 * D), _BF),
        pltpu.VMEM((8, 6 * D), _F32),
        pltpu.VMEM((S, D), _BF),
        pltpu.VMEM((D, D), _BF),
        pltpu.VMEM((D, D), _BF),
        pltpu.VMEM((nwin, S, LANES), _BF),
        pltpu.VMEM((H, VROWS, S), _BF),
        pltpu.VMEM((nblk, D, TQ), _F32),
        pltpu.VMEM((S, TQ), _F32),
        pltpu.VMEM((S, TQ), _F32),
        pltpu.VMEM((1, TQ), _F32),
        pltpu.VMEM((D, TQ), _F32),
        pltpu.SemaphoreType.DMA((10 + nblk,)),
    ]
    out = pl.pallas_call(
        functools.partial(_kernel, S=S, D=D, F=F),
        grid=(nblk,),
        in_specs=[hbm] * 8,
        out_specs=pl.BlockSpec((TQ, D), lambda i: (i, 0)),
        out_shape=jax.ShapeDtypeStruct((S, D), A_x.dtype),
        scratch_shapes=scratch,
        compiler_params=pltpu.CompilerParams(
            dimension_semantics=("arbitrary",),
            vmem_limit_bytes=100 * 1024 * 1024,
        ),
    )(x2, A_wqkv, A_wo, B_w_gate.T, B_w_up.T, B_w_down, c, w_mod)
    return out.reshape(B, S, D)
```

```python
import functools
import math

import jax
import jax.numpy as jnp
import jax.experimental.pallas as pl
import jax.experimental.pallas.tpu as pltpu

H = 32
DH = 20
EPS = 1e-5
LANES = 128
HEADS_PER_WIN = 6
VROWS = 32
TQ = 512
CK = 128
LAG = 4
FC = 512
NH = 8
KOFF = 16
PIN = 4

_BF = jnp.bfloat16
_F32 = jnp.float32
_NT = (((1,), (1,)), ((), ()))


def _layernorm(x):
    m = jnp.mean(x, axis=-1, keepdims=True)
    xc = x - m
    v = jnp.mean(xc * xc, axis=-1, keepdims=True)
    return xc * jax.lax.rsqrt(v + EPS)


def _gelu_tanh(x):
    c = math.sqrt(2.0 / math.pi)
    return 0.5 * x * (1.0 + jnp.tanh(c * (x + 0.044715 * (x * x * x))))


def _win_start(g, d_model):
    return min(g * HEADS_PER_WIN * DH, d_model - LANES)


def _kernel(x_hbm, wqkv_hbm, wo_hbm, wg_hbm, wu_hbm, wd_hbm, c_hbm, wmod_hbm,
            o_ref,
            x_v, wq_v, wk_v, wv_v, wo_v, wg_v, wu_v, wd_v, c_v, wma_v, wmb_v,
            mod_v, h_v, wqt_v, wvt_v, k_v, vt_v, qt_v,
            sa_v, sb_v, ma_v, ot_v, sems,
            *, S, D, F):
    step = pl.program_id(0)
    nblk = S // TQ
    nch = S // CK
    nwin = -(-H // HEADS_PER_WIN)
    qscale = (DH ** -0.5) * math.log2(math.e)

    def cp_c():
        return pltpu.make_async_copy(c_hbm, c_v, sems.at[0])

    def cp_wk():
        return pltpu.make_async_copy(wqkv_hbm.at[:, pl.ds(D, D)], wk_v, sems.at[1])

    def cp_wq():
        return pltpu.make_async_copy(wqkv_hbm.at[:, pl.ds(0, D)], wq_v, sems.at[8 + nblk])

    def cp_wv():
        return pltpu.make_async_copy(wqkv_hbm.at[:, pl.ds(2 * D, D)], wv_v, sems.at[9 + nblk])

    def cp_mod_a():
        return pltpu.make_async_copy(wmod_hbm.at[:, pl.ds(0, 2 * D)], wma_v, sems.at[2])

    def cp_mod_b():
        return pltpu.make_async_copy(wmod_hbm.at[:, pl.ds(2 * D, 4 * D)], wmb_v, sems.at[3])

    def cp_late():
        pairs = [(wo_hbm, wo_v), (wg_hbm, wg_v), (wu_hbm, wu_v), (wd_hbm, wd_v)]
        return [pltpu.make_async_copy(s, d, sems.at[4 + i]) for i, (s, d) in enumerate(pairs)]

    def cp_x(b):
        r0 = pl.multiple_of(b * TQ, TQ)
        return pltpu.make_async_copy(x_hbm.at[pl.ds(r0, TQ)], x_v.at[pl.ds(r0, TQ)], sems.at[8 + b])

    def qmask(blk, head):
        g = head // HEADS_PER_WIN
        start = jnp.minimum(g * (HEADS_PER_WIN * DH), D - LANES)
        base = head * DH - start
        qt = qt_v[blk, pl.ds(pl.multiple_of(start, 8), LANES), :]
        row = jax.lax.broadcasted_iota(jnp.int32, (LANES, TQ), 0)
        qm = jnp.where((row >= base) & (row < base + DH), qt, 0.0).astype(_BF)
        return g, qm

    def qk_chunk(g, qm, c, s_ref, mpart):
        rows = slice(c * CK, (c + 1) * CK)
        kb0 = pl.multiple_of(g * S + KOFF, 16)
        s = jnp.dot(k_v[pl.ds(kb0 + c * CK, CK), :], qm, preferred_element_type=_F32)
        s_ref[rows, :] = s
        mp = jnp.max(s.reshape(CK // 8, 8, TQ), axis=0)
        return mp if mpart is None else jnp.maximum(mpart, mp)

    @pl.when(step == 0)
    def _prologue():
        cp_c().start()
        cp_mod_a().start()
        cp_x(0).start()
        cp_wk().start()
        cp_c().wait()
        cp_mod_a().wait()
        c = c_v[...].astype(_F32)
        sc8 = jnp.broadcast_to((c * jax.nn.sigmoid(c)).astype(_BF), (8, D))
        mod_v[:, 0:2 * D] = jnp.dot(sc8, wma_v[...], preferred_element_type=_F32)
        shift = mod_v[0:1, 0:D]
        scale = 1.0 + mod_v[0:1, D:2 * D]
        cp_wk().wait()
        for b in range(1, nblk):
            cp_x(b).start()
        cp_wq().start()
        cp_wv().start()
        cp_mod_b().start()
        for cp in cp_late():
            cp.start()

        def proj_k(b, carry):
            cp_x(b).wait()
            for hf in range(2):
                r0 = pl.multiple_of(b * TQ + hf * (TQ // 2), TQ // 2)
                rows = pl.ds(r0, TQ // 2)
                x = x_v[rows, :].astype(_F32)
                h = (_layernorm(x) * scale + shift).astype(_BF)
                h_v[rows, :] = h
                kk = jnp.dot(h, wk_v[...], preferred_element_type=_F32)
                for g in range(nwin):
                    st = _win_start(g, D)
                    k_v[pl.ds(pl.multiple_of(g * S + KOFF + r0, 16), TQ // 2), :] = kk[:, st:st + LANES].astype(_BF)
            return carry

        jax.lax.fori_loop(0, nblk, proj_k, 0)

        cp_wq().wait()
        cp_wv().wait()
        cp_mod_b().wait()
        wqt_v[...] = wq_v[...].T
        wvt_v[...] = wv_v[...].T
        mod_v[:, 2 * D:6 * D] = jnp.dot(sc8, wmb_v[...], preferred_element_type=_F32)

        def proj_qv(b, carry):
            r0 = pl.multiple_of(b * TQ, TQ)
            h = h_v[pl.ds(r0, TQ), :]
            qt = jax.lax.dot_general(wqt_v[...], h, _NT, preferred_element_type=_F32)
            qt_v[b] = qt * qscale
            vt = jax.lax.dot_general(wvt_v[...], h, _NT, preferred_element_type=_F32)
            rowi = jax.lax.broadcasted_iota(jnp.int32, (VROWS - DH, TQ), 0)
            tail = jnp.where(rowi == 0, 1.0, 0.0).astype(_F32)
            for hh in range(H):
                slab = jnp.concatenate([vt[hh * DH:(hh + 1) * DH], tail], axis=0)
                vt_v[hh, :, pl.ds(r0, TQ)] = slab.astype(_BF)
            return carry

        jax.lax.fori_loop(0, nblk, proj_qv, 0)
        g, qm = qmask(0, 0)
        mpart = None
        for c_ in range(nch):
            mpart = qk_chunk(g, qm, c_, sa_v, mpart)
        ma_v[...] = jnp.max(mpart, axis=0, keepdims=True)
        for cp in cp_late():
            cp.wait()

    def heads(j, carry):
        h0 = NH * j
        sw = [sb_v, sa_v] * (NH // 2)
        sr = [sa_v, sb_v] * (NH // 2)
        qk = [None] * NH
        m = [ma_v[...]] + [None] * (NH - 1)
        mpart = [None] * NH
        acc = [None] * NH
        pins = {}
        pv_at = {}
        for i in range(NH):
            for c_ in range(nch):
                t = i * nch + LAG + (c_ if i < NH - 1 else (c_ * (nch - LAG)) // nch)
                pv_at.setdefault(t, []).append((i, c_))
        for t in range(NH * nch):
            i, c_ = divmod(t, nch)
            if c_ == 0:
                nxt = h0 + 1 + i
                if i == NH - 1:
                    wrap = nxt // H
                    qk[i] = qmask(jnp.minimum(step + wrap, nblk - 1), nxt - wrap * H)
                else:
                    qk[i] = qmask(step, nxt)
            mpart[i] = qk_chunk(qk[i][0], qk[i][1], c_, sw[i], mpart[i])
            if i < NH - 1:
                pins[t] = mpart[i]
            if c_ == nch - 1:
                mfin = jnp.max(mpart[i], axis=0, keepdims=True)
                if i < NH - 1:
                    m[i + 1] = mfin
                else:
                    ma_v[...] = mfin
            for i, c_ in pv_at.get(t, []):
                rows = slice(c_ * CK, (c_ + 1) * CK)
                mu = m[i]
                if (t - PIN) in pins:
                    mu = jnp.maximum(mu, jnp.minimum(pins[t - PIN][0:1, :], mu))
                p = jnp.exp2(sr[i][rows, :] - mu).astype(_BF)
                part = jnp.dot(vt_v[h0 + i, :, rows], p, preferred_element_type=_F32)
                acc[i] = part if acc[i] is None else acc[i] + part
                if c_ == nch - 1 and i % 2 == 1:
                    oa = acc[i - 1][0:DH] / acc[i - 1][DH:DH + 1]
                    ob = acc[i][0:DH] / acc[i][DH:DH + 1]
                    ot_v[pl.ds(pl.multiple_of(DH * (h0 + i - 1), 8), 2 * DH), :] = jnp.concatenate([oa, ob], axis=0)
        return carry

    jax.lax.fori_loop(0, H // NH, heads, 0)

    HT = TQ // 2
    ga = mod_v[0:1, 2 * D:3 * D]
    shift2 = mod_v[0:1, 3 * D:4 * D]
    scale2 = 1.0 + mod_v[0:1, 4 * D:5 * D]
    gb = mod_v[0:1, 5 * D:6 * D]
    x1 = []
    h2 = []
    for hf in range(2):
        r0 = pl.multiple_of(step * TQ + hf * HT, HT)
        o = ot_v[:, hf * HT:(hf + 1) * HT].T.astype(_BF)
        attn = jnp.dot(o, wo_v[...], preferred_element_type=_F32)
        xh = x_v[pl.ds(r0, HT), :].astype(_F32) + ga * attn
        x1.append(xh)
        h2.append((_layernorm(xh) * scale2 + shift2).astype(_BF))

    def gate_up(hh, f0, f1):
        gate = jax.lax.dot_general(hh, wg_v[f0:f1, :], _NT, preferred_element_type=_F32)
        up = jax.lax.dot_general(hh, wu_v[f0:f1, :], _NT, preferred_element_type=_F32)
        return (_gelu_tanh(gate) * up).astype(_BF)

    bounds = list(range(0, F, FC)) + [F]
    h2f = jnp.concatenate(h2, axis=0)
    acts = []
    for ci in range(len(bounds) - 1):
        f0, f1 = bounds[ci], bounds[ci + 1]
        if ci == 0:
            act = jnp.concatenate([gate_up(h2[0], f0, f1), gate_up(h2[1], f0, f1)], axis=0)
        elif (f1 - f0) % LANES == LANES // 2:
            fm = f1 - LANES // 2
            wt = jnp.concatenate([wg_v[fm:f1, :], wu_v[fm:f1, :]], axis=0)
            gu = jax.lax.dot_general(h2f, wt, _NT, preferred_element_type=_F32)
            tail = (_gelu_tanh(gu[:, 0:LANES // 2]) * gu[:, LANES // 2:LANES]).astype(_BF)
            act = jnp.concatenate([gate_up(h2f, f0, fm), tail], axis=1)
        else:
            act = gate_up(h2f, f0, f1)
        acts.append(act)
    acc = None
    for ci in range(len(bounds) - 2):
        part = jnp.dot(acts[ci], wd_v[bounds[ci]:bounds[ci + 1], :], preferred_element_type=_F32)
        acc = part if acc is None else acc + part
    for hf in range(2):
        rs = slice(hf * HT, (hf + 1) * HT)
        part = jnp.dot(acts[-1][rs], wd_v[bounds[-2]:bounds[-1], :], preferred_element_type=_F32)
        o_ref[rs, :] = (x1[hf] + gb * (acc[rs] + part)).astype(o_ref.dtype)


@jax.jit
def pallas_adaLN_cond__mha_block__geglu_ffn__prompt_kernel(
    A_x: jax.Array,
    A_wqkv: jax.Array,
    A_wo: jax.Array,
    B_x: jax.Array,
    B_w_gate: jax.Array,
    B_w_up: jax.Array,
    B_w_down: jax.Array,
    c: jax.Array,
    w_mod: jax.Array,
):
    B, S, D = A_x.shape
    F = B_w_gate.shape[1]
    assert B == 1 and D == H * DH and S % TQ == 0
    nblk = S // TQ
    nwin = -(-H // HEADS_PER_WIN)
    x2 = A_x.reshape(S, D)

    hbm = pl.BlockSpec(memory_space=pltpu.HBM)
    scratch = [
        pltpu.VMEM((S, D), _BF),
        pltpu.VMEM((D, D), _BF),
        pltpu.VMEM((D, D), _BF),
        pltpu.VMEM((D, D), _BF),
        pltpu.VMEM((D, D), _BF),
        pltpu.VMEM((F, D), _BF),
        pltpu.VMEM((F, D), _BF),
        pltpu.VMEM((F, D), _BF),
        pltpu.VMEM((1, D), _BF),
        pltpu.VMEM((D, 2 * D), _BF),
        pltpu.VMEM((D, 4 * D), _BF),
        pltpu.VMEM((8, 6 * D), _F32),
        pltpu.VMEM((S, D), _BF),
        pltpu.VMEM((D, D), _BF),
        pltpu.VMEM((D, D), _BF),
        pltpu.VMEM((nwin * S + 128, LANES), _BF),
        pltpu.VMEM((H, VROWS, S + LANES), _BF),
        pltpu.VMEM((nblk, D, TQ), _F32),
        pltpu.VMEM((S, TQ), _F32),
        pltpu.VMEM((S, TQ), _F32),
        pltpu.VMEM((1, TQ), _F32),
        pltpu.VMEM((D, TQ), _F32),
        pltpu.SemaphoreType.DMA((10 + nblk,)),
    ]
    out = pl.pallas_call(
        functools.partial(_kernel, S=S, D=D, F=F),
        grid=(nblk,),
        in_specs=[hbm] * 8,
        out_specs=pl.BlockSpec((TQ, D), lambda i: (i, 0)),
        out_shape=jax.ShapeDtypeStruct((S, D), A_x.dtype),
        scratch_shapes=scratch,
        compiler_params=pltpu.CompilerParams(
            dimension_semantics=("arbitrary",),
            vmem_limit_bytes=100 * 1024 * 1024,
        ),
    )(x2, A_wqkv, A_wo, B_w_gate.T, B_w_up.T, B_w_down, c, w_mod)
    return out.reshape(B, S, D)
```
